```python
import jax
import jax.numpy as jnp

def _softmax(x, axis=-1):
    return jax.nn.softmax(x, axis=axis)

def _gelu(x):
    return jax.nn.gelu(x, approximate=True)

def _silu(x):
    return jax.nn.silu(x)

def _sigmoid(x):
    return jax.nn.sigmoid(x)

def _layernorm(x, axis=-1, eps=1e-05):
    m = jnp.mean(x, axis=axis, keepdims=True)
    v = jnp.var(x, axis=axis, keepdims=True)
    return (x - m) / jnp.sqrt(v + eps)

def _scatter_add(tgt, idx, src, axis=0):
    return tgt.at[idx].add(src)

def _segment_sum(src, seg, n):
    return jax.ops.segment_sum(src, seg, n)

class _Rng:

    def __init__(self, key):
        self._k = key

    def _next(self):
        self._k, sub = jax.random.split(self._k)
        return sub

    def normal(self, shape):
        return jax.random.normal(self._next(), shape, dtype=jnp.bfloat16)

    def randint(self, lo, hi, shape):
        return jax.random.randint(self._next(), shape, lo, hi, dtype=jnp.int32)

    def uniform(self, shape, lo=0.0, hi=1.0):
        return jax.random.uniform(self._next(), shape, jnp.bfloat16, lo, hi)

    def permutation(self, n):
        return jax.random.permutation(self._next(), n)
kernel_name = 'concat_heads__sliding_local_dilated__memory_aug_recurrent_mem_tr__prompt'

def setup_inputs():
    _rng = _Rng(jax.random.key(int.from_bytes(__import__("os").urandom(4), "little")))
    _w = lambda a: (lambda t: t.astype(jnp.bfloat16) if jnp.issubdtype(t.dtype, jnp.floating) else t)(jnp.asarray(a))

    def _A_setup():
        B, S, D = (1, 2048, 640)
        return {'x': _w((lambda *s: _rng.normal(s) * 0.05)(B, S, D)), 'wqkv': _w((lambda *s: _rng.normal(s) * 0.05)(D, 3 * D)), 'wo': _w((lambda *s: _rng.normal(s) * 0.05)(D, D))}
    _A_in = _A_setup()

    def _B_setup():
        B, S, Dm = (1, 2048, 640)
        H, Dh = (32, 192)
        M, seg = (8, 32)
        seg = min(seg, S)
        S = S // seg * seg
        return {'x': _w((lambda *s: _rng.normal(s) * 0.05)(B, S, Dm)), 'mem0': _w((lambda *s: _rng.normal(s) * 0.05)(B, M, Dm)), 'Wq': _w((lambda *s: _rng.normal(s) * 0.05)(Dm, H, Dh) * Dm ** (-0.5)), 'Wk': _w((lambda *s: _rng.normal(s) * 0.05)(Dm, H, Dh) * Dm ** (-0.5)), 'Wv': _w((lambda *s: _rng.normal(s) * 0.05)(Dm, H, Dh) * Dm ** (-0.5)), 'Wo': _w((lambda *s: _rng.normal(s) * 0.05)(H, Dh, Dm) * (H * Dh) ** (-0.5)), 'seg_len': seg}
    _B_in = _B_setup()
    return {'A_x': _A_in['x'], 'A_wqkv': _A_in['wqkv'], 'A_wo': _A_in['wo'], 'B_x': _B_in['x'], 'B_mem0': _B_in['mem0'], 'B_Wq': _B_in['Wq'], 'B_Wk': _B_in['Wk'], 'B_Wv': _B_in['Wv'], 'B_Wo': _B_in['Wo'], 'B_seg_len': _B_in['seg_len']}

def reference(A_x, A_wqkv, A_wo, B_x, B_mem0, B_Wq, B_Wk, B_Wv, B_Wo, B_seg_len):

    def _A_ref(x, wqkv, wo):
        B, S, D = x.shape
        H = 32
        Dh = D // H
        W, dil = (8, 2)
        qkv = (lambda x, *d: x.transpose(*d))((x @ wqkv).reshape(B, S, 3, H, Dh), 2, 0, 3, 1, 4)
        q, k, v = (qkv[0], qkv[1], qkv[2])
        scale = Dh ** (-0.5)
        pos = jnp.arange(S)
        off = jnp.arange(W) * dil
        idx = pos[:, None] - off[None, :]
        mask = idx >= 0
        idx_c = jnp.where(mask, idx, 0).reshape(-1)
        kg = k[:, :, idx_c, :].reshape(B, H, S, W, Dh)
        vg = v[:, :, idx_c, :].reshape(B, H, S, W, Dh)
        logits = jnp.einsum('bhsd,bhswd->bhsw', q, kg) * scale
        logits = jnp.where(mask[None, None, :, :], logits, -1000000000.0)
        attn = _softmax(logits, axis=-1)
        o = jnp.einsum('bhsw,bhswd->bhsd', attn, vg)
        return (lambda x, *d: x.transpose(*d))(o, 0, 2, 1, 3).reshape(B, S, D) @ wo

    def _B_ref(x, mem0, Wq, Wk, Wv, Wo, seg_len):
        B, S, Dm = x.shape
        H, Dh = (Wq.shape[1], Wq.shape[2])
        M = mem0.shape[1]
        scale = Dh ** (-0.5)
        n_seg = S // seg_len
        L = M + seg_len
        idx = jnp.arange(L)
        mask = (idx[:, None] < M) | (idx[:, None] >= idx[None, :])
        mem = mem0
        outs = []
        for s in range(n_seg):
            xs = x[:, s * seg_len:(s + 1) * seg_len, :].copy()
            h = jnp.concatenate([mem, xs], axis=1)
            q = jnp.einsum('btd,dhe->bhte', h, Wq)
            k = jnp.einsum('btd,dhe->bhte', h, Wk)
            v = jnp.einsum('btd,dhe->bhte', h, Wv)
            scores = jnp.einsum('bhqe,bhke->bhqk', q, k) * scale
            scores = jnp.where(mask[None, None], scores, -1000000000.0)
            p = _softmax(scores, axis=-1)
            o = jnp.einsum('bhqk,bhke->bhqe', p, v)
            o = jnp.einsum('bhte,hed->btd', o, Wo)
            mem = o[:, :M, :].copy()
            outs.append(o[:, M:, :])
        return jnp.concatenate(outs, axis=1)
    a = _A_ref(A_x, A_wqkv, A_wo)
    b = _B_ref(B_x, B_mem0, B_Wq, B_Wk, B_Wv, B_Wo, B_seg_len)
    return jnp.concatenate([a, b], axis=-1)
```

```python
import functools
import math

import jax
import jax.numpy as jnp
import jax.experimental.pallas as pl
import jax.experimental.pallas.tpu as pltpu

F32, BF16, U32 = jnp.float32, jnp.bfloat16, jnp.uint32
NN = (((1,), (0,)), ((), ()))
NT = (((1,), (1,)), ((), ()))
LANES = 128
NEG = -1000000000.0
LOG2E = math.log2(math.e)

A_HEADS, A_WIN, A_DIL = 32, 8, 2
A_HALO = 16
A_ROWS = 128


def _dot(a, b, dims):
    return jax.lax.dot_general(a, b, dims, preferred_element_type=F32)


def _kernel(xa_hbm, wqkv_hbm, woa_hbm, xb_hbm, mem0_hbm, wq_hbm, wk_hbm, wv_hbm, wob_hbm,
            out_hbm,
            xa, wqkv, woa, xb, mem0, wstage, wob,
            ptmp, wqkv_t, woa_p, q0, q1, kv0, kv1, oa, wb, ob, outa, outb,
            sem_in, sem_w, sem_out,
            *, seq, dm, heads_b, dh_b, n_mem, seg):
    R = A_ROWS
    n_blk = seq // R
    n_ct = dm // LANES
    dh_a = dm // A_HEADS
    n_pair = heads_b // 2
    pw = 2 * dh_b
    pairs_per_blk = n_pair // n_blk
    L = n_mem + seg
    n_seg = seq // seg

    cp_wqkv = pltpu.make_async_copy(wqkv_hbm, wqkv, sem_in.at[0])
    cp_xa = pltpu.make_async_copy(xa_hbm, xa, sem_in.at[1])
    cp_woa = pltpu.make_async_copy(woa_hbm, woa, sem_in.at[2])
    cp_wob = pltpu.make_async_copy(wob_hbm, wob, sem_in.at[3])
    cp_xb = pltpu.make_async_copy(xb_hbm, xb, sem_in.at[4])
    cp_mem0 = pltpu.make_async_copy(mem0_hbm, mem0, sem_in.at[5])

    def cp_w(j, m):
        src = (wq_hbm, wk_hbm, wv_hbm)[m]
        r = j * pw if isinstance(j, int) else pl.multiple_of(j * pw, pw)
        return pltpu.make_async_copy(src.at[pl.ds(r, pw), :], wstage.at[j, m], sem_w.at[j * 3 + m])

    cp_wqkv.start()
    cp_xa.start()
    cp_woa.start()
    cp_wqkv.wait()
    for j in range(n_pair):
        for m in range(3):
            cp_w(j, m).start()
    cp_wob.start()
    cp_xb.start()
    cp_mem0.start()

    def permute_rows(t, dst, row0, col):
        for d in range(dh_a):
            dst[pl.ds(row0 + d * A_HEADS, A_HEADS), pl.ds(col * LANES, LANES)] = (
                ptmp[t, pl.ds(d, A_HEADS, stride=dh_a), :].astype(BF16))

    for p in range(3):
        for c in range(n_ct):
            ptmp[p * n_ct + c] = wqkv[pl.ds(c * LANES, LANES), pl.ds(p * dm, dm)].astype(F32).T
            permute_rows(p * n_ct + c, wqkv_t, p * dm, c)
    cp_woa.wait()
    for c in range(n_ct):
        ptmp[3 * n_ct + c] = woa[:, pl.ds(c * LANES, LANES)].astype(F32)
        permute_rows(3 * n_ct + c, woa_p, 0, c)
    cp_xa.wait()

    q_mul = dh_a ** -0.5 * LOG2E
    G = 8

    def blk_rows(b):
        return pl.ds(b * R if isinstance(b, int) else pl.multiple_of(b * R, R), R)

    def a_proj(x, t, q_dst, kv_dst):
        y = _dot(x, wqkv_t[pl.ds(t * LANES, LANES), :], NT)
        if t < n_ct:
            q_dst[t] = y * q_mul
        else:
            kv_dst[t - n_ct, pl.ds(A_HALO, R), :] = y

    def a_attend(g, q_src, kv_src, first_block):
        r = g * G
        q = [q_src[c, pl.ds(r, G), :] for c in range(n_ct)]
        s = []
        for w in range(A_WIN):
            rows = pl.ds(A_HALO + r - w * A_DIL, G)
            t = q[0] * kv_src[0, rows, :]
            for c in range(1, n_ct):
                t = t + q[c] * kv_src[c, rows, :]
            t = t + pltpu.roll(t, 2 * A_HEADS, 1)
            t = t + pltpu.roll(t, A_HEADS, 1)
            if first_block and r < w * A_DIL:
                pos = r + jax.lax.broadcasted_iota(jnp.int32, (G, LANES), 0)
                t = jnp.where(pos >= w * A_DIL, t, NEG * LOG2E)
            s.append(t)
        m = functools.reduce(jnp.maximum, s)
        p = [jnp.exp2(t - m) for t in s]
        inv = 1.0 / functools.reduce(jnp.add, p)
        for c in range(n_ct):
            o = p[0] * kv_src[n_ct + c, pl.ds(A_HALO + r, G), :]
            for w in range(1, A_WIN):
                o = o + p[w] * kv_src[n_ct + c, pl.ds(A_HALO + r - w * A_DIL, G), :]
            oa[pl.ds(r, G), pl.ds(c * LANES, LANES)] = o * inv

    def b_relayout(j, m):
        wb[j, :, pl.ds(m * pw, pw)] = pltpu.bitcast(wstage[j, m].T, U32)

    def a_stage(b, cur, nxt, first_block, project_next):
        (q_cur, kv_cur), (q_nxt, kv_nxt) = cur, nxt
        n_g, n_t = R // G, 3 * n_ct
        relayouts = [(b * pairs_per_blk + i, m) for i in range(pairs_per_blk) for m in range(3)]
        if project_next:
            x = xa[blk_rows(b + 1), :]
            kv_nxt[:, pl.ds(0, A_HALO), :] = kv_cur[:, pl.ds(R, A_HALO), :]
        done_g = 0
        for t in range(n_t):
            if project_next:
                a_proj(x, t, q_nxt, kv_nxt)
            while done_g < min(n_g, ((t + 1) * n_g + 11) // 12):
                a_attend(done_g, q_cur, kv_cur, first_block)
                done_g += 1
            if t % 5 == 2 and relayouts:
                for _ in range(pairs_per_blk):
                    b_relayout(*relayouts.pop(0))
        outa[blk_rows(b), :] = _dot(oa[...], woa_p[...], NN).astype(BF16)

    def wait_pairs(b0, nb):
        for i in range(nb * pairs_per_blk):
            for m in range(3):
                cp_w(b0 * pairs_per_blk + i, m).wait()

    buf0, buf1 = (q0, kv0), (q1, kv1)
    x0 = xa[blk_rows(0), :]
    for t in range(3 * n_ct):
        a_proj(x0, t, q0, kv0)
    kv0[:, pl.ds(0, A_HALO), :] = jnp.broadcast_to(
        kv0[:, pl.ds(A_HALO, 1), :], (2 * n_ct, A_HALO, LANES))
    wait_pairs(0, 1)
    a_stage(0, buf0, buf1, True, True)

    def a_loop(i, carry):
        b = 2 * i + 1
        wait_pairs(b, 2)
        a_stage(b, buf1, buf0, False, True)
        a_stage(b + 1, buf0, buf1, False, True)
        return carry

    jax.lax.fori_loop(0, (n_blk - 2) // 2, a_loop, 0)
    wait_pairs(n_blk - 1, 1)
    a_stage(n_blk - 1, buf1, buf0, False, False)

    cp_wob.wait()
    cp_xb.wait()
    cp_mem0.wait()
    cp_outa = pltpu.make_async_copy(outa, out_hbm.at[:, pl.ds(0, dm)], sem_out.at[0])
    cp_outa.start()

    s_mul = dh_b ** -0.5 * LOG2E
    low_half = jax.lax.broadcasted_iota(jnp.int32, (L, LANES), 1) < dh_b - LANES
    row = jax.lax.broadcasted_iota(jnp.int32, (L, 2 * L), 0)
    col = jax.lax.broadcasted_iota(jnp.int32, (L, 2 * L), 1)
    head0 = col < L
    visible = (row < n_mem) | (row >= jnp.where(head0, col, col - L))

    def block_diag(t):
        t0, t1, t2 = (t[:, i * LANES:(i + 1) * LANES] for i in range(3))
        z = jnp.zeros_like(t0)
        top = jnp.concatenate([t0, jnp.where(low_half, t1, 0.0), z], axis=1)
        bot = jnp.concatenate([z, jnp.where(low_half, 0.0, t1), t2], axis=1)
        return jnp.concatenate([top, bot], axis=0).astype(BF16)

    def pair_softmax(s):
        s = jnp.where(visible, s * s_mul, NEG * LOG2E)
        m0 = jnp.max(jnp.where(head0, s, -jnp.inf), axis=1, keepdims=True)
        m1 = jnp.max(jnp.where(head0, -jnp.inf, s), axis=1, keepdims=True)
        p = jnp.exp2(s - jnp.where(head0, m0, m1))
        l0 = jnp.sum(jnp.where(head0, p, 0.0), axis=1, keepdims=True)
        l1 = jnp.sum(jnp.where(head0, 0.0, p), axis=1, keepdims=True)
        return p * (1.0 / jnp.where(head0, l0, l1))

    lag_s, lag_p, o_chunk = 1, 3, 2

    def seg_rows(s):
        return pl.ds(pl.multiple_of(s * seg, seg), seg)

    def b_step(s, mem):
        h = jnp.concatenate([mem, xb[seg_rows(s), :].astype(F32)], axis=0)
        proj, prob, out, next_o = {}, {}, None, 0

        def out_proj(acc, i):
            c = pl.ds(i * o_chunk * pw, o_chunk * pw)
            d = _dot(ob[:, c], wob[c, :], NN)
            return d if acc is None else acc + d

        for t in range(n_pair + lag_p):
            if t < n_pair:
                y = _dot(h, pltpu.bitcast(wb[t], BF16), NN)
                proj[t] = y[:, :pw], block_diag(y[:, pw:2 * pw]), block_diag(y[:, 2 * pw:])
            else:
                out = out_proj(out, next_o)
                next_o += 1
            if 0 <= t - lag_s < n_pair:
                q, k, _ = proj[t - lag_s]
                prob[t - lag_s] = pair_softmax(_dot(q, k, NT))
            if 0 <= t - lag_p < n_pair:
                j = t - lag_p
                ob[:, pl.ds(j * pw, pw)] = _dot(prob[j], proj[j][2], NN)
        for i in range(next_o, n_pair // o_chunk):
            out = out_proj(out, i)
        outb[seg_rows(s), :] = out[n_mem:].astype(BF16)
        pltpu.make_async_copy(
            outb.at[seg_rows(s), :], out_hbm.at[seg_rows(s), pl.ds(dm, dm)], sem_out.at[1]).start()
        return out[:n_mem].astype(BF16).astype(F32)

    jax.lax.fori_loop(0, n_seg, b_step, mem0[...].astype(F32))
    cp_outa.wait()
    pltpu.make_async_copy(outb, out_hbm.at[:, pl.ds(dm, dm)], sem_out.at[1]).wait()


@functools.partial(jax.jit, static_argnames=("B_seg_len",))
def pallas_concat_heads__sliding_local_dilated__memory_aug_recurrent_mem_tr__prompt_kernel(
    A_x: jax.Array,
    A_wqkv: jax.Array,
    A_wo: jax.Array,
    B_x: jax.Array,
    B_mem0: jax.Array,
    B_Wq: jax.Array,
    B_Wk: jax.Array,
    B_Wv: jax.Array,
    B_Wo: jax.Array,
    B_seg_len: int,
):
    _, seq, dm = A_x.shape
    _, heads_b, dh_b = B_Wq.shape
    n_mem = B_mem0.shape[1]
    seg = int(B_seg_len)
    hd = heads_b * dh_b
    pw = 2 * dh_b
    n_pair = heads_b // 2
    n_ct = dm // LANES
    assert A_x.shape[0] == 1 and B_x.shape == A_x.shape
    assert LANES == 4 * A_HEADS and dm % LANES == 0 and pw == 3 * LANES
    assert seq % (2 * A_ROWS) == 0 and n_pair % (seq // A_ROWS) == 0
    assert seq % seg == 0 and seg % 16 == 0 and n_mem % 8 == 0 and 2 * (n_mem + seg) <= LANES

    rows_major = lambda w: jnp.transpose(w, (1, 2, 0)).reshape(hd, dm)

    vmem = pltpu.VMEM
    out = pl.pallas_call(
        functools.partial(_kernel, seq=seq, dm=dm, heads_b=heads_b, dh_b=dh_b, n_mem=n_mem, seg=seg),
        out_shape=jax.ShapeDtypeStruct((seq, 2 * dm), BF16),
        in_specs=[pl.BlockSpec(memory_space=pl.ANY)] * 9,
        out_specs=pl.BlockSpec(memory_space=pl.ANY),
        scratch_shapes=[
            vmem((seq, dm), BF16),
            vmem((dm, 3 * dm), BF16),
            vmem((dm, dm), BF16),
            vmem((seq, dm), BF16),
            vmem((n_mem, dm), BF16),
            vmem((n_pair, 3, pw, dm), BF16),
            vmem((hd, dm), BF16),
            vmem((4 * n_ct, dm, LANES), F32),
            vmem((3 * dm, dm), BF16),
            vmem((dm, dm), BF16),
            vmem((n_ct, A_ROWS, LANES), F32),
            vmem((n_ct, A_ROWS, LANES), F32),
            vmem((2 * n_ct, A_HALO + A_ROWS, LANES), F32),
            vmem((2 * n_ct, A_HALO + A_ROWS, LANES), F32),
            vmem((A_ROWS, dm), F32),
            vmem((n_pair, dm // 2, 3 * pw), U32),
            vmem((n_mem + seg, hd), F32),
            vmem((seq, dm), BF16),
            vmem((seq, dm), BF16),
            pltpu.SemaphoreType.DMA((6,)),
            pltpu.SemaphoreType.DMA((3 * n_pair,)),
            pltpu.SemaphoreType.DMA((2,)),
        ],
        compiler_params=pltpu.CompilerParams(vmem_limit_bytes=110 * 1024 * 1024),
    )(
        A_x.reshape(seq, dm), A_wqkv, A_wo,
        B_x.reshape(seq, dm), B_mem0.reshape(n_mem, dm),
        rows_major(B_Wq), rows_major(B_Wk), rows_major(B_Wv), B_Wo.reshape(hd, dm),
    )
    return out.reshape(1, seq, 2 * dm)
```

```python
import functools
import math

import jax
import jax.numpy as jnp
import jax.experimental.pallas as pl
import jax.experimental.pallas.tpu as pltpu

F32, BF16, U32 = jnp.float32, jnp.bfloat16, jnp.uint32
NN = (((1,), (0,)), ((), ()))
NT = (((1,), (1,)), ((), ()))
LANES = 128
NEG = -1000000000.0
LOG2E = math.log2(math.e)

A_HEADS, A_WIN, A_DIL = 32, 8, 2
A_HALO = 16
A_ROWS = 64
A_STAGES = 4
A_SPREAD = 12
B_EARLY = 4
B_UNROLL = 1
LAG_QK, LAG_PV = 1, 3
O_PAIRS = 2
WO_PAIRS = 8


def _dot(a, b, dims):
    return jax.lax.dot_general(a, b, dims, preferred_element_type=F32)


def _kernel(xa_hbm, wqkv_hbm, woa_hbm, xb_hbm, mem0_hbm, wq_hbm, wk_hbm, wv_hbm, wob_hbm,
            out_hbm,
            xa, wqkv, woa, xb, mem0, wstage, wob,
            ptmp, wqkv_p, woa_p, q0, q1, kv0, kv1, oa, wb, ob, outa, outb,
            sem_in, sem_a, sem_x, sem_w, sem_o, sem_out,
            *, seq, dm, heads_b, dh_b, n_mem, seg):
    R = A_ROWS
    n_blk = seq // R
    n_ct = dm // LANES
    dh_a = dm // A_HEADS
    n_pair = heads_b // 2
    pw = 2 * dh_b
    L = n_mem + seg
    n_seg = seq // seg
    n_iter = n_blk // A_STAGES
    pairs_per_iter = n_pair // n_iter
    n_oc = n_pair // O_PAIRS

    def rows_copy(src, dst, row0, n, sem):
        if not isinstance(row0, int):
            row0 = pl.multiple_of(row0, 16)
        return pltpu.make_async_copy(src.at[pl.ds(row0, n), :], dst.at[pl.ds(row0, n), :], sem)

    cp_wqkv = [rows_copy(wqkv_hbm, wqkv, c * LANES, LANES, sem_a.at[c]) for c in range(n_ct)]
    cp_woa = pltpu.make_async_copy(woa_hbm, woa, sem_in.at[0])
    cp_xb0 = rows_copy(xb_hbm, xb, 0, B_EARLY * seg, sem_in.at[1])
    cp_xb1 = rows_copy(xb_hbm, xb, B_EARLY * seg, seq - B_EARLY * seg, sem_in.at[2])
    cp_mem0 = pltpu.make_async_copy(mem0_hbm, mem0, sem_in.at[3])
    cp_wob = [rows_copy(wob_hbm, wob, i * WO_PAIRS * pw, WO_PAIRS * pw, sem_o.at[i])
              for i in range(n_pair // WO_PAIRS)]

    def cp_xa(i):
        return rows_copy(xa_hbm, xa, i * A_STAGES * R, A_STAGES * R, sem_x.at[i])

    def pairs_of(i):
        return [(i * pairs_per_iter + j, m) for j in range(pairs_per_iter) for m in range(3)]

    def cp_w(j, m):
        src = (wq_hbm, wk_hbm, wv_hbm)[m]
        return pltpu.make_async_copy(
            src.at[pl.ds(pl.multiple_of(j * pw, pw), pw), :], wstage.at[j, m], sem_w.at[j * 3 + m])

    def start_iter_inputs(i, carry):
        pl.when(i + 1 < n_iter)(lambda: cp_xa(i + 1).start())
        for j, m in pairs_of(i):
            cp_w(j, m).start()
        return carry

    dma_groups = [
        lambda: [cp_xa(0).start(), cp_woa.start()],
        lambda: jax.lax.fori_loop(0, n_iter, start_iter_inputs, 0),
        lambda: [cp.start() for cp in (cp_xb0, cp_mem0)],
        lambda: [cp.start() for cp in cp_wob],
        lambda: cp_xb1.start(),
    ]
    for cp in cp_wqkv:
        cp.start()

    def permuted_rows(t):
        return jnp.concatenate(
            [ptmp[t, pl.ds(d, A_HEADS, stride=dh_a), :].astype(BF16) for d in range(dh_a)], axis=0)

    for c in range(n_ct):
        cp_wqkv[c].wait()
        dma_groups[c]()
        for p in range(3):
            ptmp[p] = wqkv[pl.ds(c * LANES, LANES), pl.ds(p * dm, dm)].astype(F32).T
            wqkv_p[pl.ds(c * LANES // 2, LANES // 2), pl.ds(p * dm, dm)] = pltpu.bitcast(
                permuted_rows(p).T, U32)
    cp_xa(0).wait()

    q_mul = dh_a ** -0.5 * LOG2E
    G = 8

    def blk_rows(b):
        return pl.ds(b * R if isinstance(b, int) else pl.multiple_of(b * R, R), R)

    def a_proj(x, t, q_dst, kv_dst):
        y = _dot(x, pltpu.bitcast(wqkv_p[:, pl.ds(t * LANES, LANES)], BF16), NN)
        if t < n_ct:
            q_dst[t] = y * q_mul
        else:
            kv_dst[t - n_ct, pl.ds(A_HALO, R), :] = y

    def a_attend(g, q_src, kv_src, block0):
        r = g * G
        q = [q_src[c, pl.ds(r, G), :] for c in range(n_ct)]
        pos = block0 + r + jax.lax.broadcasted_iota(jnp.int32, (G, LANES), 0)
        s = []
        for w in range(A_WIN):
            rows = pl.ds(A_HALO + r - w * A_DIL, G)
            t = q[0] * kv_src[0, rows, :]
            for c in range(1, n_ct):
                t = t + q[c] * kv_src[c, rows, :]
            t = t + pltpu.roll(t, 2 * A_HEADS, 1)
            t = t + pltpu.roll(t, A_HEADS, 1)
            if r < w * A_DIL:
                t = jnp.where(pos >= w * A_DIL, t, NEG * LOG2E)
            s.append(t)
        m = functools.reduce(jnp.maximum, s)
        p = [jnp.exp2(t - m) for t in s]
        inv = 1.0 / functools.reduce(jnp.add, p)
        for c in range(n_ct):
            o = p[0] * kv_src[n_ct + c, pl.ds(A_HALO + r, G), :]
            for w in range(1, A_WIN):
                o = o + p[w] * kv_src[n_ct + c, pl.ds(A_HALO + r - w * A_DIL, G), :]
            oa[pl.ds(r, G), pl.ds(c * LANES, LANES)] = o * inv

    def b_relayout(j, m):
        wb[j, :, pl.ds(m * pw, pw)] = pltpu.bitcast(wstage[j, m].T, U32)

    def a_stage(b, cur, nxt, relayouts):
        (q_cur, kv_cur), (q_nxt, kv_nxt) = cur, nxt
        n_g, n_t, n_r = R // G, 3 * n_ct, len(relayouts)
        x = xa[blk_rows(jnp.minimum(b + 1, n_blk - 1)), :]
        kv_nxt[:, pl.ds(0, A_HALO), :] = kv_cur[:, pl.ds(R, A_HALO), :]
        done_g = done_r = 0
        for t in range(n_t):
            a_proj(x, t, q_nxt, kv_nxt)
            while done_g < min(n_g, ((t + 1) * n_g + A_SPREAD - 1) // A_SPREAD):
                a_attend(done_g, q_cur, kv_cur, b * R)
                done_g += 1
            while done_r < ((t + 3) * n_r) // (n_t + 2):
                b_relayout(*relayouts[done_r])
                done_r += 1
        outa[blk_rows(b), :] = _dot(oa[...], pltpu.bitcast(woa_p[...], BF16), NN).astype(BF16)

    bufs = (q0, kv0), (q1, kv1)
    x0 = xa[blk_rows(0), :]
    for t in range(3 * n_ct):
        a_proj(x0, t, q0, kv0)
    kv0[:, pl.ds(0, A_HALO), :] = jnp.broadcast_to(
        kv0[:, pl.ds(A_HALO, 1), :], (2 * n_ct, A_HALO, LANES))
    cp_woa.wait()
    for c in range(n_ct):
        ptmp[c] = woa[:, pl.ds(c * LANES, LANES)].astype(F32)
        woa_p[:, pl.ds(c * LANES, LANES)] = pltpu.bitcast(permuted_rows(c), U32)

    def a_loop(i, carry):
        todo = pairs_of(i)
        pl.when(i + 1 < n_iter)(lambda: cp_xa(i + 1).wait())
        for j, m in todo:
            cp_w(j, m).wait()
        for k in range(A_STAGES):
            mine = todo[k * len(todo) // A_STAGES:(k + 1) * len(todo) // A_STAGES]
            a_stage(i * A_STAGES + k, bufs[k % 2], bufs[1 - k % 2], mine)
        return carry

    jax.lax.fori_loop(0, n_iter, a_loop, 0)
    cp_xb0.wait()
    cp_mem0.wait()

    s_mul = dh_b ** -0.5 * LOG2E
    low_half = jax.lax.broadcasted_iota(jnp.int32, (L, LANES), 1) < dh_b - LANES
    row = jax.lax.broadcasted_iota(jnp.int32, (L, 2 * L), 0)
    col = jax.lax.broadcasted_iota(jnp.int32, (L, 2 * L), 1)
    head0 = col < L
    visible = (row < n_mem) | (row >= jnp.where(head0, col, col - L))

    def block_diag(t):
        t0, t1, t2 = (t[:, i * LANES:(i + 1) * LANES] for i in range(3))
        z = jnp.zeros_like(t0)
        top = jnp.concatenate([t0, jnp.where(low_half, t1, 0.0), z], axis=1)
        bot = jnp.concatenate([z, jnp.where(low_half, 0.0, t1), t2], axis=1)
        return jnp.concatenate([top, bot], axis=0).astype(BF16)

    def pair_softmax(s):
        s = jnp.where(visible, s * s_mul, NEG * LOG2E)
        m0 = jnp.max(jnp.where(head0, s, -jnp.inf), axis=1, keepdims=True)
        m1 = jnp.max(jnp.where(head0, -jnp.inf, s), axis=1, keepdims=True)
        p = jnp.exp2(s - jnp.where(head0, m0, m1))
        l0 = jnp.sum(jnp.where(head0, p, 0.0), axis=1, keepdims=True)
        l1 = jnp.sum(jnp.where(head0, 0.0, p), axis=1, keepdims=True)
        return p * (1.0 / jnp.where(head0, l0, l1))

    def seg_rows(s):
        return pl.ds(s * seg if isinstance(s, int) else pl.multiple_of(s * seg, seg), seg)

    def b_step(s, mem, first=False):
        h = jnp.concatenate([mem, xb[seg_rows(s), :].astype(F32)], axis=0)
        proj, prob, out, next_o = {}, {}, None, 0

        def out_proj(acc, i):
            if first and i * O_PAIRS % WO_PAIRS == 0:
                cp_wob[i * O_PAIRS // WO_PAIRS].wait()
            c = pl.ds(i * O_PAIRS * pw, O_PAIRS * pw)
            d = _dot(ob[:, c], wob[c, :], NN)
            return d if acc is None else acc + d

        for t in range(n_pair + LAG_PV):
            if t < n_pair:
                y = _dot(h, pltpu.bitcast(wb[t], BF16), NN)
                proj[t] = y[:, :pw], block_diag(y[:, pw:2 * pw]), block_diag(y[:, 2 * pw:])
            else:
                out = out_proj(out, next_o)
                next_o += 1
            if 0 <= t - LAG_QK < n_pair:
                q, k, _ = proj[t - LAG_QK]
                prob[t - LAG_QK] = pair_softmax(_dot(q, k, NT))
            if 0 <= t - LAG_PV < n_pair:
                j = t - LAG_PV
                ob[:, pl.ds(j * pw, pw)] = _dot(prob[j], proj[j][2], NN)
        for i in range(next_o, n_oc):
            out = out_proj(out, i)
        outb[seg_rows(s), :] = out[n_mem:].astype(BF16)
        pltpu.make_async_copy(
            outb.at[seg_rows(s), :], out_hbm.at[seg_rows(s), pl.ds(dm, dm)], sem_out.at[1]).start()
        return out[:n_mem].astype(BF16).astype(F32)

    mem1 = b_step(0, mem0[...].astype(F32), first=True)
    cp_outa = pltpu.make_async_copy(outa, out_hbm.at[:, pl.ds(0, dm)], sem_out.at[0])
    cp_outa.start()

    def b_loop(i, mem):
        s = 1 + i * B_UNROLL
        pl.when(i == (B_EARLY - 1) // B_UNROLL)(cp_xb1.wait)
        for k in range(B_UNROLL):
            mem = b_step(s + k, mem)
        return mem

    jax.lax.fori_loop(0, (n_seg - 1) // B_UNROLL, b_loop, mem1)
    cp_outa.wait()
    pltpu.make_async_copy(outb, out_hbm.at[:, pl.ds(dm, dm)], sem_out.at[1]).wait()


@functools.partial(jax.jit, static_argnames=("B_seg_len",))
def pallas_concat_heads__sliding_local_dilated__memory_aug_recurrent_mem_tr__prompt_kernel(
    A_x: jax.Array,
    A_wqkv: jax.Array,
    A_wo: jax.Array,
    B_x: jax.Array,
    B_mem0: jax.Array,
    B_Wq: jax.Array,
    B_Wk: jax.Array,
    B_Wv: jax.Array,
    B_Wo: jax.Array,
    B_seg_len: int,
):
    _, seq, dm = A_x.shape
    _, heads_b, dh_b = B_Wq.shape
    n_mem = B_mem0.shape[1]
    seg = int(B_seg_len)
    hd = heads_b * dh_b
    pw = 2 * dh_b
    n_pair = heads_b // 2
    n_ct = dm // LANES
    assert A_x.shape[0] == 1 and B_x.shape == A_x.shape
    assert LANES == 4 * A_HEADS and dm == 5 * LANES and pw == 3 * LANES
    assert seq % (A_STAGES * A_ROWS) == 0 and n_pair % (seq // (A_STAGES * A_ROWS)) == 0
    assert (seq // seg - 1) % B_UNROLL == 0
    assert seq % seg == 0 and seg % 16 == 0 and n_mem % 8 == 0 and 2 * (n_mem + seg) <= LANES

    rows_major = lambda w: jnp.transpose(w, (1, 2, 0)).reshape(hd, dm)

    vmem = pltpu.VMEM
    out = pl.pallas_call(
        functools.partial(_kernel, seq=seq, dm=dm, heads_b=heads_b, dh_b=dh_b, n_mem=n_mem, seg=seg),
        out_shape=jax.ShapeDtypeStruct((seq, 2 * dm), BF16),
        in_specs=[pl.BlockSpec(memory_space=pl.ANY)] * 9,
        out_specs=pl.BlockSpec(memory_space=pl.ANY),
        scratch_shapes=[
            vmem((seq, dm), BF16),
            vmem((dm, 3 * dm), BF16),
            vmem((dm, dm), BF16),
            vmem((seq, dm), BF16),
            vmem((n_mem, dm), BF16),
            vmem((n_pair, 3, pw, dm), BF16),
            vmem((hd, dm), BF16),
            vmem((n_ct, dm, LANES), F32),
            vmem((dm // 2, 3 * dm), U32),
            vmem((dm // 2, dm), U32),
            vmem((n_ct, A_ROWS, LANES), F32),
            vmem((n_ct, A_ROWS, LANES), F32),
            vmem((2 * n_ct, A_HALO + A_ROWS, LANES), F32),
            vmem((2 * n_ct, A_HALO + A_ROWS, LANES), F32),
            vmem((A_ROWS, dm), F32),
            vmem((n_pair, dm // 2, 3 * pw), U32),
            vmem((n_mem + seg, hd), F32),
            vmem((seq, dm), BF16),
            vmem((seq, dm), BF16),
            pltpu.SemaphoreType.DMA((4,)),
            pltpu.SemaphoreType.DMA((n_ct,)),
            pltpu.SemaphoreType.DMA((seq // (A_STAGES * A_ROWS),)),
            pltpu.SemaphoreType.DMA((3 * n_pair,)),
            pltpu.SemaphoreType.DMA((n_pair // WO_PAIRS,)),
            pltpu.SemaphoreType.DMA((2,)),
        ],
        compiler_params=pltpu.CompilerParams(vmem_limit_bytes=110 * 1024 * 1024),
    )(
        A_x.reshape(seq, dm), A_wqkv, A_wo,
        B_x.reshape(seq, dm), B_mem0.reshape(n_mem, dm),
        rows_major(B_Wq), rows_major(B_Wk), rows_major(B_Wv), B_Wo.reshape(hd, dm),
    )
    return out.reshape(1, seq, 2 * dm)
```

```python
import functools
import math

import jax
import jax.numpy as jnp
import jax.experimental.pallas as pl
import jax.experimental.pallas.tpu as pltpu

F32, BF16, U32 = jnp.float32, jnp.bfloat16, jnp.uint32
NN = (((1,), (0,)), ((), ()))
NT = (((1,), (1,)), ((), ()))
LANES = 128
NEG = -1000000000.0
LOG2E = math.log2(math.e)

A_HEADS, A_WIN, A_DIL = 32, 8, 2
A_HALO = 16
A_ROWS = 64
A_STAGES = 2
A_OROWS = 32
A_GROUP = 16
B_EARLY = 4
B_UNROLL = 3
LAG_QK, LAG_PV = 1, 3
O_PAIRS = 2
WO_PAIRS = 8


def _dot(a, b, dims):
    return jax.lax.dot_general(a, b, dims, preferred_element_type=F32)


def _kernel(xa_hbm, wqkv_hbm, woa_hbm, xb_hbm, mem0_hbm, wq_hbm, wk_hbm, wv_hbm, wob_hbm,
            out_hbm,
            xa, wqkv, woa, xb, mem0, wstage, wob,
            ptmp, wqkv_p, woa_p, q0, q1, kv0, kv1, oa, wb, ob, outa, outb,
            sem_in, sem_a, sem_x, sem_w, sem_o, sem_out,
            *, seq, dm, heads_b, dh_b, n_mem, seg):
    R = A_ROWS
    n_blk = seq // R
    n_ct = dm // LANES
    dh_a = dm // A_HEADS
    n_pair = heads_b // 2
    pw = 2 * dh_b
    L = n_mem + seg
    n_seg = seq // seg
    n_iter = n_blk // A_STAGES
    pairs_per_iter = n_pair // n_iter
    n_oc = n_pair // O_PAIRS

    def rows_copy(src, dst, row0, n, sem):
        if not isinstance(row0, int):
            row0 = pl.multiple_of(row0, 16)
        return pltpu.make_async_copy(src.at[pl.ds(row0, n), :], dst.at[pl.ds(row0, n), :], sem)

    cp_wqkv = [rows_copy(wqkv_hbm, wqkv, c * LANES, LANES, sem_a.at[c]) for c in range(n_ct)]
    cp_woa = pltpu.make_async_copy(woa_hbm, woa, sem_in.at[0])
    cp_xb0 = rows_copy(xb_hbm, xb, 0, B_EARLY * seg, sem_in.at[1])
    cp_xb1 = rows_copy(xb_hbm, xb, B_EARLY * seg, seq - B_EARLY * seg, sem_in.at[2])
    cp_mem0 = pltpu.make_async_copy(mem0_hbm, mem0, sem_in.at[3])
    cp_wob = [rows_copy(wob_hbm, wob, i * WO_PAIRS * pw, WO_PAIRS * pw, sem_o.at[i])
              for i in range(n_pair // WO_PAIRS)]

    def cp_xa(i):
        return rows_copy(xa_hbm, xa, i * A_STAGES * R, A_STAGES * R, sem_x.at[i])

    def slots_of(i):
        return [(i * pairs_per_iter + j, m) for j in range(pairs_per_iter) for m in range(3)]

    def cp_w(slot, m):
        j = slot - pairs_per_iter
        src = (wq_hbm, wk_hbm, wv_hbm)[m]
        r = j * pw if isinstance(j, int) else pl.multiple_of(j * pw, pw)
        return pltpu.make_async_copy(src.at[pl.ds(r, pw), :], wstage.at[slot, m], sem_w.at[j])

    def wait_slots(i):
        for slot, m in slots_of(i):
            cp_w(slot, m).wait()

    def start_iter_inputs(i, carry):
        pl.when(i + 1 < n_iter)(lambda: cp_xa(i + 1).start())
        for slot, m in slots_of(i + 1):
            cp_w(slot, m).start()
        return carry

    dma_groups = [
        lambda: [cp_xa(0).start(), cp_woa.start()],
        lambda: jax.lax.fori_loop(0, n_iter, start_iter_inputs, 0),
        lambda: [cp.start() for cp in (cp_xb0, cp_mem0)],
        lambda: [cp.start() for cp in cp_wob],
        lambda: cp_xb1.start(),
    ]
    for cp in cp_wqkv:
        cp.start()

    def permuted_rows(t):
        return jnp.concatenate(
            [ptmp[t, pl.ds(d, A_HEADS, stride=dh_a), :].astype(BF16) for d in range(dh_a)], axis=0)

    for c in range(n_ct):
        cp_wqkv[c].wait()
        dma_groups[c]()
        for p in range(3):
            ptmp[p] = wqkv[pl.ds(c * LANES, LANES), pl.ds(p * dm, dm)].astype(F32).T
            wqkv_p[pl.ds(c * LANES // 2, LANES // 2), pl.ds(p * dm, dm)] = pltpu.bitcast(
                permuted_rows(p).T, U32)
    cp_xa(0).wait()
    cp_woa.wait()
    for c in range(n_ct):
        ptmp[c] = woa[:, pl.ds(c * LANES, LANES)].astype(F32)
        woa_p[:, pl.ds(c * LANES, LANES)] = pltpu.bitcast(permuted_rows(c), U32)

    q_mul = dh_a ** -0.5 * LOG2E
    G, OR = A_GROUP, A_OROWS

    def blk_rows(b):
        return pl.ds(b * R if isinstance(b, int) else pl.multiple_of(b * R, R), R)

    def a_proj(x, t, q_dst, kv_dst):
        y = _dot(x, pltpu.bitcast(wqkv_p[:, pl.ds(t * LANES, LANES)], BF16), NN)
        if t < n_ct:
            q_dst[t] = y * q_mul
        else:
            kv_dst[t - n_ct, pl.ds(A_HALO, R), :] = y

    def a_attend(g, q_src, kv_src, block0):
        r = g * G
        q = [q_src[c, pl.ds(r, G), :] for c in range(n_ct)]
        pos = block0 + r + jax.lax.broadcasted_iota(jnp.int32, (G, LANES), 0)
        s = []
        for w in range(A_WIN):
            rows = pl.ds(A_HALO + r - w * A_DIL, G)
            t = q[0] * kv_src[0, rows, :]
            for c in range(1, n_ct):
                t = t + q[c] * kv_src[c, rows, :]
            t = t + pltpu.roll(t, 2 * A_HEADS, 1)
            t = t + pltpu.roll(t, A_HEADS, 1)
            if r < w * A_DIL:
                t = jnp.where(pos >= w * A_DIL, t, NEG * LOG2E)
            s.append(t)
        m = functools.reduce(jnp.maximum, s)
        p = [jnp.exp2(t - m) for t in s]
        inv = 1.0 / functools.reduce(jnp.add, p)
        for c in range(n_ct):
            o = p[0] * kv_src[n_ct + c, pl.ds(A_HALO + r, G), :]
            for w in range(1, A_WIN):
                o = o + p[w] * kv_src[n_ct + c, pl.ds(A_HALO + r - w * A_DIL, G), :]
            oa[pl.ds(r, G), pl.ds(c * LANES, LANES)] = (o * inv).astype(BF16)

    def b_relayout(j, m):
        wb[j, :, pl.ds(m * pw, pw)] = pltpu.bitcast(wstage[j, m].T, U32)

    def a_stage(b, cur, nxt, relayouts):
        (q_cur, kv_cur), (q_nxt, kv_nxt) = cur, nxt
        n_t, n_r = 3 * n_ct, len(relayouts)
        x = xa[blk_rows(jnp.minimum(b + 1, n_blk - 1)), :]
        kv_nxt[:, pl.ds(0, A_HALO), :] = kv_cur[:, pl.ds(R, A_HALO), :]
        done_r = 0
        n_o = R // OR
        for t in range(n_t):
            a_proj(x, t, q_nxt, kv_nxt)
            while done_r < ((t + 3) * n_r) // (n_t + 2):
                b_relayout(*relayouts[done_r])
                done_r += 1
            for i in range(n_o):
                if t == (i + 1) * n_t // n_o - 1:
                    for g in range(i * OR // G, (i + 1) * OR // G):
                        a_attend(g, q_cur, kv_cur, b * R)
                    outa[pl.ds(pl.multiple_of(b * R + i * OR, OR), OR), :] = _dot(
                        oa[pl.ds(i * OR, OR), :], pltpu.bitcast(woa_p[...], BF16), NN).astype(BF16)

    bufs = (q0, kv0), (q1, kv1)
    x0 = xa[blk_rows(0), :]
    for t in range(3 * n_ct):
        a_proj(x0, t, q0, kv0)
    kv0[:, pl.ds(0, A_HALO), :] = jnp.broadcast_to(
        kv0[:, pl.ds(A_HALO, 1), :], (2 * n_ct, A_HALO, LANES))

    def a_loop(i, carry):
        todo = slots_of(i)
        pl.when(i + 1 < n_iter)(lambda: cp_xa(i + 1).wait())
        pl.when(i > 0)(lambda: wait_slots(i))
        for k in range(A_STAGES):
            mine = todo[k * len(todo) // A_STAGES:(k + 1) * len(todo) // A_STAGES]
            a_stage(i * A_STAGES + k, bufs[k % 2], bufs[1 - k % 2], mine)
        return carry

    jax.lax.fori_loop(0, n_iter, a_loop, 0)
    cp_xb0.wait()
    cp_mem0.wait()
    wait_slots(n_iter)
    for slot, m in slots_of(n_iter):
        b_relayout(slot, m)

    s_mul = dh_b ** -0.5 * LOG2E
    low_half = jax.lax.broadcasted_iota(jnp.int32, (L, LANES), 1) < dh_b - LANES
    row = jax.lax.broadcasted_iota(jnp.int32, (L, 2 * L), 0)
    col = jax.lax.broadcasted_iota(jnp.int32, (L, 2 * L), 1)
    head0 = col < L
    visible = (row < n_mem) | (row >= jnp.where(head0, col, col - L))

    def block_diag(t):
        t0, t1, t2 = (t[:, i * LANES:(i + 1) * LANES] for i in range(3))
        z = jnp.zeros_like(t0)
        top = jnp.concatenate([t0, jnp.where(low_half, t1, 0.0), z], axis=1)
        bot = jnp.concatenate([z, jnp.where(low_half, 0.0, t1), t2], axis=1)
        return jnp.concatenate([top, bot], axis=0).astype(BF16)

    def pair_softmax(s):
        s = jnp.where(visible, s * s_mul, NEG * LOG2E)
        m0 = jnp.max(jnp.where(head0, s, -jnp.inf), axis=1, keepdims=True)
        m1 = jnp.max(jnp.where(head0, -jnp.inf, s), axis=1, keepdims=True)
        p = jnp.exp2(s - jnp.where(head0, m0, m1))
        l0 = jnp.sum(jnp.where(head0, p, 0.0), axis=1, keepdims=True)
        l1 = jnp.sum(jnp.where(head0, 0.0, p), axis=1, keepdims=True)
        return p * (1.0 / jnp.where(head0, l0, l1))

    def seg_rows(s):
        return pl.ds(s * seg if isinstance(s, int) else pl.multiple_of(s * seg, seg), seg)

    def b_step(s, mem, first=False):
        h = jnp.concatenate([mem, xb[seg_rows(s), :].astype(F32)], axis=0)
        proj, prob, out, next_o = {}, {}, None, 0

        def out_proj(acc, i):
            if first and i * O_PAIRS % WO_PAIRS == 0:
                cp_wob[i * O_PAIRS // WO_PAIRS].wait()
            c = pl.ds(i * O_PAIRS * pw, O_PAIRS * pw)
            d = _dot(ob[:, c], wob[c, :], NN)
            return d if acc is None else acc + d

        for t in range(n_pair + LAG_PV):
            if t < n_pair:
                y = _dot(h, pltpu.bitcast(wb[t + pairs_per_iter], BF16), NN)
                proj[t] = y[:, :pw], block_diag(y[:, pw:2 * pw]), block_diag(y[:, 2 * pw:])
            else:
                out = out_proj(out, next_o)
                next_o += 1
            if 0 <= t - LAG_QK < n_pair:
                q, k, _ = proj[t - LAG_QK]
                prob[t - LAG_QK] = pair_softmax(_dot(q, k, NT))
            if 0 <= t - LAG_PV < n_pair:
                j = t - LAG_PV
                ob[:, pl.ds(j * pw, pw)] = _dot(prob[j], proj[j][2], NN)
        for i in range(next_o, n_oc):
            out = out_proj(out, i)
        outb[seg_rows(s), :] = out[n_mem:].astype(BF16)
        pltpu.make_async_copy(
            outb.at[seg_rows(s), :], out_hbm.at[seg_rows(s), pl.ds(dm, dm)], sem_out.at[1]).start()
        return out[:n_mem].astype(BF16).astype(F32)

    mem1 = b_step(0, mem0[...].astype(F32), first=True)
    cp_outa = pltpu.make_async_copy(outa, out_hbm.at[:, pl.ds(0, dm)], sem_out.at[0])
    cp_outa.start()

    def b_loop(i, mem):
        s = 1 + i * B_UNROLL
        pl.when(i == (B_EARLY - 1) // B_UNROLL)(cp_xb1.wait)
        for k in range(B_UNROLL):
            mem = b_step(s + k, mem)
        return mem

    jax.lax.fori_loop(0, (n_seg - 1) // B_UNROLL, b_loop, mem1)
    cp_outa.wait()
    pltpu.make_async_copy(outb, out_hbm.at[:, pl.ds(dm, dm)], sem_out.at[1]).wait()


@functools.partial(jax.jit, static_argnames=("B_seg_len",))
def pallas_concat_heads__sliding_local_dilated__memory_aug_recurrent_mem_tr__prompt_kernel(
    A_x: jax.Array,
    A_wqkv: jax.Array,
    A_wo: jax.Array,
    B_x: jax.Array,
    B_mem0: jax.Array,
    B_Wq: jax.Array,
    B_Wk: jax.Array,
    B_Wv: jax.Array,
    B_Wo: jax.Array,
    B_seg_len: int,
):
    _, seq, dm = A_x.shape
    _, heads_b, dh_b = B_Wq.shape
    n_mem = B_mem0.shape[1]
    seg = int(B_seg_len)
    hd = heads_b * dh_b
    pw = 2 * dh_b
    n_pair = heads_b // 2
    n_ct = dm // LANES
    n_iter = seq // (A_STAGES * A_ROWS)
    n_slot = n_pair + n_pair // n_iter
    assert A_x.shape[0] == 1 and B_x.shape == A_x.shape
    assert LANES == 4 * A_HEADS and dm == 5 * LANES and pw == 3 * LANES
    assert seq % (A_STAGES * A_ROWS) == 0 and n_pair % n_iter == 0
    assert (seq // seg - 1) % B_UNROLL == 0
    assert seq % seg == 0 and seg % 16 == 0 and n_mem % 8 == 0 and 2 * (n_mem + seg) <= LANES

    rows_major = lambda w: jnp.transpose(w, (1, 2, 0)).reshape(hd, dm)

    vmem = pltpu.VMEM
    out = pl.pallas_call(
        functools.partial(_kernel, seq=seq, dm=dm, heads_b=heads_b, dh_b=dh_b, n_mem=n_mem, seg=seg),
        out_shape=jax.ShapeDtypeStruct((seq, 2 * dm), BF16),
        in_specs=[pl.BlockSpec(memory_space=pl.ANY)] * 9,
        out_specs=pl.BlockSpec(memory_space=pl.ANY),
        scratch_shapes=[
            vmem((seq, dm), BF16),
            vmem((dm, 3 * dm), BF16),
            vmem((dm, dm), BF16),
            vmem((seq, dm), BF16),
            vmem((n_mem, dm), BF16),
            vmem((n_slot, 3, pw, dm), BF16),
            vmem((hd, dm), BF16),
            vmem((n_ct, dm, LANES), F32),
            vmem((dm // 2, 3 * dm), U32),
            vmem((dm // 2, dm), U32),
            vmem((n_ct, A_ROWS, LANES), F32),
            vmem((n_ct, A_ROWS, LANES), F32),
            vmem((2 * n_ct, A_HALO + A_ROWS, LANES), F32),
            vmem((2 * n_ct, A_HALO + A_ROWS, LANES), F32),
            vmem((A_ROWS, dm), BF16),
            vmem((n_slot, dm // 2, 3 * pw), U32),
            vmem((n_mem + seg, hd), F32),
            vmem((seq, dm), BF16),
            vmem((seq, dm), BF16),
            pltpu.SemaphoreType.DMA((4,)),
            pltpu.SemaphoreType.DMA((n_ct,)),
            pltpu.SemaphoreType.DMA((n_iter,)),
            pltpu.SemaphoreType.DMA((n_pair,)),
            pltpu.SemaphoreType.DMA((n_pair // WO_PAIRS,)),
            pltpu.SemaphoreType.DMA((2,)),
        ],
        compiler_params=pltpu.CompilerParams(vmem_limit_bytes=110 * 1024 * 1024),
    )(
        A_x.reshape(seq, dm), A_wqkv, A_wo,
        B_x.reshape(seq, dm), B_mem0.reshape(n_mem, dm),
        rows_major(B_Wq), rows_major(B_Wk), rows_major(B_Wv), B_Wo.reshape(hd, dm),
    )
    return out.reshape(1, seq, 2 * dm)
```

```python
import functools
import math

import jax
import jax.numpy as jnp
import jax.experimental.pallas as pl
import jax.experimental.pallas.tpu as pltpu

F32, BF16, U32 = jnp.float32, jnp.bfloat16, jnp.uint32
NN = (((1,), (0,)), ((), ()))
NT = (((1,), (1,)), ((), ()))
LANES = 128
LOG2E = math.log2(math.e)
MASKED = -1000000000.0 * LOG2E

A_HEADS, A_WIN, A_DIL = 32, 8, 2

A_HALO = 16
A_ROWS = 64
A_OUT_ROWS = 32
A_GROUP = 16

B_UNROLL = 3
B_EARLY = 4
LAG_QK, LAG_PV = 1, 3
O_CHUNKS = (2, 2, 2, 2, 4, 4)
WO_PAIRS = 8


def _dot(a, b, dims=NN):
    return jax.lax.dot_general(a, b, dims, preferred_element_type=F32)


def _rows(i, n):
    return pl.ds(i * n if isinstance(i, int) else pl.multiple_of(i * n, n), n)


def _unpack(w):
    return pltpu.bitcast(w, BF16)


def _kernel(xa_hbm, wqkv_hbm, woa_hbm, xb_hbm, mem0_hbm, wq_hbm, wk_hbm, wv_hbm, wob_hbm,
            out_hbm,
            xa, wqkv, woa, xb, mem0, wstage, wob,
            ptmp, wqkv_p, woa_p, q0, q1, kv0, kv1, oa, wb, ob, outa, outb,
            sem_in, sem_a, sem_x, sem_w, sem_o, sem_out,
            *, seg):
    seq, dm = xa.shape
    n_pair, _, pw, _ = wstage.shape
    n_mem = mem0.shape[0]
    dh_a, dh_b = dm // A_HEADS, pw // 2
    n_ct = dm // LANES
    R, G = A_ROWS, A_GROUP
    n_blk = seq // R
    L = n_mem + seg

    def copy(src, dst, rows, sem):
        return pltpu.make_async_copy(src.at[rows, :], dst.at[rows, :], sem)

    cp_wqkv = [copy(wqkv_hbm, wqkv, _rows(c, LANES), sem_a.at[c]) for c in range(n_ct)]
    cp_woa = pltpu.make_async_copy(woa_hbm, woa, sem_in.at[0])
    cp_mem0 = pltpu.make_async_copy(mem0_hbm, mem0, sem_in.at[1])
    cp_xb_early = copy(xb_hbm, xb, pl.ds(0, B_EARLY * seg), sem_in.at[2])
    cp_xb_rest = copy(xb_hbm, xb, pl.ds(B_EARLY * seg, seq - B_EARLY * seg), sem_in.at[3])
    cp_wob = [copy(wob_hbm, wob, _rows(i, WO_PAIRS * pw), sem_o.at[i])
              for i in range(n_pair // WO_PAIRS)]
    cp_outa = pltpu.make_async_copy(outa, out_hbm.at[:, pl.ds(0, dm)], sem_out.at[0])

    def cp_xa(i):
        return copy(xa_hbm, xa, _rows(i, 2 * R), sem_x.at[i])

    def cp_pair(j):
        return [pltpu.make_async_copy(w.at[_rows(j, pw), :], wstage.at[j, m], sem_w.at[j])
                for m, w in enumerate((wq_hbm, wk_hbm, wv_hbm))]

    def start(copies):
        for cp in copies:
            cp.start()

    def wait(copies):
        for cp in copies:
            cp.wait()

    def start_phase_a_inputs():
        @pl.loop(1, n_pair)
        def _(i):
            start([cp_xa(i)] + cp_pair(i - 1))
        start(cp_pair(n_pair - 1))

    copy_groups = [
        lambda: start([cp_xa(0), cp_woa]),
        start_phase_a_inputs,
        lambda: start([cp_xb_early, cp_mem0]),
        lambda: start(cp_wob),
        lambda: start([cp_xb_rest]),
    ]
    start(cp_wqkv)

    def permuted_rows(t):
        return jnp.concatenate(
            [ptmp[t, pl.ds(d, A_HEADS, stride=dh_a), :].astype(BF16) for d in range(dh_a)], axis=0)

    for c in range(n_ct):
        cp_wqkv[c].wait()
        copy_groups[c]()
        for p in range(3):
            ptmp[p] = wqkv[_rows(c, LANES), _rows(p, dm)].astype(F32).T
            wqkv_p[_rows(c, LANES // 2), _rows(p, dm)] = pltpu.bitcast(permuted_rows(p).T, U32)
    wait([cp_xa(0), cp_woa])
    for c in range(n_ct):
        ptmp[c] = woa[:, _rows(c, LANES)].astype(F32)
        woa_p[:, _rows(c, LANES)] = pltpu.bitcast(permuted_rows(c), U32)

    def a_project(x, t, q_dst, kv_dst):
        y = _dot(x, _unpack(wqkv_p[:, _rows(t, LANES)]))
        if t < n_ct:
            q_dst[t] = y * (dh_a ** -0.5 * LOG2E)
        else:
            kv_dst[t - n_ct, pl.ds(A_HALO, R), :] = y

    def a_attend(r, q_src, kv_src, first_block):
        past = [pl.ds(A_HALO + r - w * A_DIL, G) for w in range(A_WIN)]
        q = [q_src[c, pl.ds(r, G), :] for c in range(n_ct)]
        s = []
        for w in range(A_WIN):
            t = functools.reduce(jnp.add, [q[c] * kv_src[c, past[w], :] for c in range(n_ct)])
            t = t + pltpu.roll(t, 2 * A_HEADS, 1)
            t = t + pltpu.roll(t, A_HEADS, 1)
            if first_block and r < w * A_DIL:
                pos = r + jax.lax.broadcasted_iota(jnp.int32, (G, LANES), 0)
                t = jnp.where(pos >= w * A_DIL, t, MASKED)
            s.append(t)
        m = functools.reduce(jnp.maximum, s)
        p = [jnp.exp2(t - m) for t in s]
        inv = 1.0 / functools.reduce(jnp.add, p)
        for c in range(n_ct):
            o = functools.reduce(
                jnp.add, [p[w] * kv_src[n_ct + c, past[w], :] for w in range(A_WIN)])
            oa[pl.ds(r, G), _rows(c, LANES)] = (o * inv).astype(BF16)

    def b_transpose(j, m):
        wb[j, :, _rows(m, pw)] = pltpu.bitcast(wstage[j, m].T, U32)

    def a_stage(b, cur, nxt, *, first_block=False, transposes=()):
        n_t, n_o = 3 * n_ct, R // A_OUT_ROWS
        if nxt is not None:
            x = xa[_rows(b + 1, R), :]
            nxt[1][:, pl.ds(0, A_HALO), :] = cur[1][:, pl.ds(R, A_HALO), :]
        for j, m in transposes:
            b_transpose(j, m)
        for i in range(n_o):
            if nxt is not None:
                for t in range(i * n_t // n_o, (i + 1) * n_t // n_o):
                    a_project(x, t, *nxt)
            for r in range(i * A_OUT_ROWS, (i + 1) * A_OUT_ROWS, G):
                a_attend(r, *cur, first_block)
            outa[_rows(b * n_o + i, A_OUT_ROWS), :] = _dot(
                oa[_rows(i, A_OUT_ROWS), :], _unpack(woa_p[...])).astype(BF16)

    even, odd = (q0, kv0), (q1, kv1)
    x0 = xa[_rows(0, R), :]
    for t in range(3 * n_ct):
        a_project(x0, t, *even)
    kv0[:, pl.ds(0, A_HALO), :] = jnp.broadcast_to(
        kv0[:, pl.ds(A_HALO, 1), :], (2 * n_ct, A_HALO, LANES))
    a_stage(0, even, odd, first_block=True)

    @pl.loop(1, n_pair)
    def _(i):
        wait([cp_xa(i)] + cp_pair(i - 1))
        a_stage(2 * i - 1, odd, even, transposes=[(i - 1, 0)])
        a_stage(2 * i, even, odd, transposes=[(i - 1, 1), (i - 1, 2)])

    wait([cp_xb_early, cp_mem0] + cp_pair(n_pair - 1))
    for m in range(3):
        b_transpose(n_pair - 1, m)

    low_half = jax.lax.broadcasted_iota(jnp.int32, (L, LANES), 1) < dh_b - LANES
    row = jax.lax.broadcasted_iota(jnp.int32, (L, 2 * L), 0)
    col = jax.lax.broadcasted_iota(jnp.int32, (L, 2 * L), 1)
    head0 = col < L
    visible = (row < n_mem) | (row >= jnp.where(head0, col, col - L))

    def block_diag(t):
        t0, t1, t2 = (t[:, i * LANES:(i + 1) * LANES] for i in range(3))
        z = jnp.zeros_like(t0)
        top = jnp.concatenate([t0, jnp.where(low_half, t1, 0.0), z], axis=1)
        bot = jnp.concatenate([z, jnp.where(low_half, 0.0, t1), t2], axis=1)
        return jnp.concatenate([top, bot], axis=0).astype(BF16)

    def pair_softmax(s):
        s = jnp.where(visible, s * (dh_b ** -0.5 * LOG2E), MASKED)
        m0 = jnp.max(jnp.where(head0, s, -jnp.inf), axis=1, keepdims=True)
        m1 = jnp.max(jnp.where(head0, -jnp.inf, s), axis=1, keepdims=True)
        p = jnp.exp2(s - jnp.where(head0, m0, m1))
        l0 = jnp.sum(jnp.where(head0, p, 0.0), axis=1, keepdims=True)
        l1 = jnp.sum(jnp.where(head0, 0.0, p), axis=1, keepdims=True)
        return p * (1.0 / jnp.where(head0, l0, l1))

    def b_project(h, j):
        if j > 0:
            y = _dot(h, _unpack(wb[j]))
        else:
            k = dm - LANES
            early = _dot(h[:, :k], _unpack(wb[j, :k // 2, :pw]))
            q = _dot(h[:, k:], _unpack(wb[j, k // 2:, :pw])) + early
            y = jnp.concatenate([q, _dot(h, _unpack(wb[j, :, pw:]))], axis=1)
        return y[:, :pw], block_diag(y[:, pw:2 * pw]), block_diag(y[:, 2 * pw:])

    def b_step(s, mem, first_step=False):
        h = jnp.concatenate([mem, xb[_rows(s, seg), :].astype(F32)], axis=0)
        qkv, prob, out = {}, {}, None
        chunks = [(sum(O_CHUNKS[:i]), n) for i, n in enumerate(O_CHUNKS)]

        def add_output_chunk(acc):
            j, n = chunks.pop(0)
            if first_step and j % WO_PAIRS == 0:
                cp_wob[j // WO_PAIRS].wait()
            d = _dot(ob[:, pl.ds(j * pw, n * pw)], wob[pl.ds(j * pw, n * pw), :])
            return d if acc is None else acc + d

        for t in range(n_pair + LAG_PV):
            if t < n_pair:
                qkv[t] = b_project(h, t)
            else:
                out = add_output_chunk(out)
            if first_step and t == 4:
                a_stage(n_blk - 1, odd, None)
            if 0 <= t - LAG_QK < n_pair:
                q, k, _ = qkv[t - LAG_QK]
                prob[t - LAG_QK] = pair_softmax(_dot(q, k, NT))
            if 0 <= t - LAG_PV < n_pair:
                ob[:, _rows(t - LAG_PV, pw)] = _dot(prob[t - LAG_PV], qkv[t - LAG_PV][2])
        while chunks:
            out = add_output_chunk(out)

        outb[_rows(s, seg), :] = out[n_mem:].astype(BF16)
        pltpu.make_async_copy(outb.at[_rows(s, seg), :], out_hbm.at[_rows(s, seg), pl.ds(dm, dm)],
                              sem_out.at[1]).start()
        return out[:n_mem].astype(BF16).astype(F32)

    def b_loop(i, mem):
        pl.when(i == (B_EARLY - 1) // B_UNROLL)(cp_xb_rest.wait)
        for k in range(B_UNROLL):
            mem = b_step(1 + i * B_UNROLL + k, mem)
        return mem

    mem1 = b_step(0, mem0[...].astype(F32), first_step=True)
    cp_outa.start()
    jax.lax.fori_loop(0, (seq // seg - 1) // B_UNROLL, b_loop, mem1)
    cp_outa.wait()
    pltpu.make_async_copy(outb, out_hbm.at[:, pl.ds(dm, dm)], sem_out.at[1]).wait()


@functools.partial(jax.jit, static_argnames=("B_seg_len",))
def pallas_concat_heads__sliding_local_dilated__memory_aug_recurrent_mem_tr__prompt_kernel(
    A_x: jax.Array,
    A_wqkv: jax.Array,
    A_wo: jax.Array,
    B_x: jax.Array,
    B_mem0: jax.Array,
    B_Wq: jax.Array,
    B_Wk: jax.Array,
    B_Wv: jax.Array,
    B_Wo: jax.Array,
    B_seg_len: int,
):
    _, seq, dm = A_x.shape
    _, heads_b, dh_b = B_Wq.shape
    n_mem, seg = B_mem0.shape[1], int(B_seg_len)
    hd, pw, n_pair, n_ct = heads_b * dh_b, 2 * dh_b, heads_b // 2, dm // LANES
    assert A_x.shape[0] == 1 and B_x.shape == A_x.shape
    assert LANES == 4 * A_HEADS and dm == 5 * LANES and pw == 3 * LANES
    assert seq == 2 * A_ROWS * n_pair and sum(O_CHUNKS) == n_pair
    assert seq % seg == 0 and (seq // seg - 1) % B_UNROLL == 0
    assert seg % 16 == 0 and n_mem % 8 == 0 and 2 * (n_mem + seg) <= LANES

    def rows_major(w):
        return jnp.transpose(w, (1, 2, 0)).reshape(hd, dm)

    vmem, dma_sems = pltpu.VMEM, pltpu.SemaphoreType.DMA
    out = pl.pallas_call(
        functools.partial(_kernel, seg=seg),
        out_shape=jax.ShapeDtypeStruct((seq, 2 * dm), BF16),
        in_specs=[pl.BlockSpec(memory_space=pl.ANY)] * 9,
        out_specs=pl.BlockSpec(memory_space=pl.ANY),
        scratch_shapes=[
            vmem((seq, dm), BF16),
            vmem((dm, 3 * dm), BF16),
            vmem((dm, dm), BF16),
            vmem((seq, dm), BF16),
            vmem((n_mem, dm), BF16),
            vmem((n_pair, 3, pw, dm), BF16),
            vmem((hd, dm), BF16),
            vmem((n_ct, dm, LANES), F32),
            vmem((dm // 2, 3 * dm), U32),
            vmem((dm // 2, dm), U32),
            vmem((n_ct, A_ROWS, LANES), F32),
            vmem((n_ct, A_ROWS, LANES), F32),
            vmem((2 * n_ct, A_HALO + A_ROWS, LANES), F32),
            vmem((2 * n_ct, A_HALO + A_ROWS, LANES), F32),
            vmem((A_ROWS, dm), BF16),
            vmem((n_pair, dm // 2, 3 * pw), U32),
            vmem((n_mem + seg, hd), F32),
            vmem((seq, dm), BF16),
            vmem((seq, dm), BF16),
            dma_sems((4,)),
            dma_sems((n_ct,)),
            dma_sems((n_pair,)),
            dma_sems((n_pair,)),
            dma_sems((n_pair // WO_PAIRS,)),
            dma_sems((2,)),
        ],
        compiler_params=pltpu.CompilerParams(vmem_limit_bytes=110 * 1024 * 1024),
    )(
        A_x.reshape(seq, dm), A_wqkv, A_wo,
        B_x.reshape(seq, dm), B_mem0.reshape(n_mem, dm),
        rows_major(B_Wq), rows_major(B_Wk), rows_major(B_Wv), B_Wo.reshape(hd, dm),
    )
    return out.reshape(1, seq, 2 * dm)
```
